```python
import os as _os
_os.environ.setdefault("JAX_PLATFORMS", "cpu")
import jax
import jax.numpy as jnp

def _softmax(x, axis=-1):
    return jax.nn.softmax(x, axis=axis)
def _gelu(x):
    return jax.nn.gelu(x, approximate=True)
def _silu(x):
    return jax.nn.silu(x)
def _sigmoid(x):
    return jax.nn.sigmoid(x)
def _layernorm(x, axis=-1, eps=1e-5):
    m = jnp.mean(x, axis=axis, keepdims=True)
    v = jnp.var(x, axis=axis, keepdims=True)
    return (x - m) / jnp.sqrt(v + eps)
def _scatter_add(tgt, idx, src, axis=0):
    return tgt.at[idx].add(src)
def _segment_sum(src, seg, n):
    return jax.ops.segment_sum(src, seg, n)
class _Rng:
    def __init__(self, key):
        self._k = key
    def _next(self):
        self._k, sub = jax.random.split(self._k)
        return sub
    def normal(self, shape):
        return jax.random.normal(self._next(), shape, dtype=jnp.bfloat16)
    def randint(self, lo, hi, shape):
        return jax.random.randint(self._next(), shape, lo, hi, dtype=jnp.int32)
    def uniform(self, shape, lo=0.0, hi=1.0):
        return jax.random.uniform(self._next(), shape, jnp.bfloat16, lo, hi)
    def permutation(self, n):
        return jax.random.permutation(self._next(), n)


kernel_name = 'gated_mix__linear_attn_block__mixer_token_mlp__prompt'

def setup_inputs():
    _rng = _Rng(jax.random.key(int.from_bytes(__import__("os").urandom(4), "little")))
    _w = (lambda a: (lambda t: t.astype(jnp.bfloat16) if jnp.issubdtype(t.dtype, jnp.floating) else t)(jnp.asarray(a)))
    def _A_setup():
        B, S, D = 1, 2048, 512
        return {
            "x": _w((lambda *s: _rng.normal(s) * 0.05)(B, S, D)),
            "wqkv": _w((lambda *s: _rng.normal(s) * 0.8)(D, 3 * D)),
            "wo": _w((lambda *s: _rng.normal(s) * 0.05)(D, D)),
        }
    _A_in = _A_setup()

    def _B_setup():
        B, S, D, F = 1, 2048, 512, 1792
        return {
            "x": _w((lambda *s: _rng.normal(s) * 0.05)(B, S, D)),
            "w1": _w((lambda *s: _rng.normal(s) * 0.1)(S, F) * (S ** -0.5)),
            "b1": _w((lambda *s: _rng.normal(s) * 0.1)(F) * 0.02),
            "w2": _w((lambda *s: _rng.normal(s) * 0.1)(F, S) * (F ** -0.5)),
            "b2": _w((lambda *s: _rng.normal(s) * 0.1)(S) * 0.02),
        }
    _B_in = _B_setup()

    return {
        "A_x": _A_in["x"],
        "A_wqkv": _A_in["wqkv"],
        "A_wo": _A_in["wo"],
        "B_x": _B_in["x"],
        "B_w1": _B_in["w1"],
        "B_b1": _B_in["b1"],
        "B_w2": _B_in["w2"],
        "B_b2": _B_in["b2"],
        "gate_w": _w((lambda *s: _rng.normal(s) * 0.05)(512) * 16.0),
    }

def reference(A_x, A_wqkv, A_wo, B_x, B_w1, B_b1, B_w2, B_b2, gate_w):
    def _A_ref(x, wqkv, wo):
        B, S, D = x.shape
        H = 32; Dh = D // H
        qkv = (lambda x, *d: x.transpose(*d))((x @ wqkv).reshape(B, S, 3, H, Dh), 2, 0, 3, 1, 4)
        q, k, v = qkv[0], qkv[1], qkv[2]
        phi = lambda t: jnp.where(t > 0, t + 1, jnp.exp(t)) + 1e-6
        pq, pk = phi(q), phi(k)
        kv = jnp.einsum("bhsd,bhse->bhde", pk, v)
        z = jnp.einsum("bhsd->bhd", pk)
        num = jnp.einsum("bhqd,bhde->bhqe", pq, kv)
        den = jnp.einsum("bhqd,bhd->bhq", pq, z)[..., None] + 1e-6
        o = num / den
        return (lambda x, *d: x.transpose(*d))(o, 0, 2, 1, 3).reshape(B, S, D) @ wo

    def _B_ref(x, w1, b1, w2, b2):
        B, S, D = x.shape
        h = _layernorm(x, axis=-1)
        u = jnp.einsum("bsd,sf->bdf", h, w1) + b1
        u = _gelu(u)
        y = jnp.einsum("bdf,fs->bds", u, w2) + b2
        return (lambda x, *d: x.transpose(*d))(y, 0, 2, 1)

    x = A_x
    g = _sigmoid((x * gate_w).sum(-1, keepdims=True))
    a = _A_ref(x, A_wqkv, A_wo)
    b = _B_ref(x, B_w1, B_b1, B_w2, B_b2)
    return g * a + (1 - g) * b
```

```python
import functools
import jax
import jax.numpy as jnp
from jax import lax
import jax.experimental.pallas as pl
import jax.experimental.pallas.tpu as pltpu

S, D, F, H, DH = 2048, 512, 1792, 32, 16
TS = 256
NS = S // TS
NG = D // 128


def _phi(t):
    return jnp.where(t > 0, t + 1.0, jnp.exp(t)) + 1e-6


def _kernel(x_ref, wqkv_ref, wo_ref, w1_ref, b1_ref, w2_ref, b2_ref, gw_ref, o_ref,
            u_acc, kv_acc, z_acc, gu_ref, kvw_ref, zmat_ref, wkT_ref):
    f32, bf16 = jnp.float32, jnp.bfloat16
    i = pl.program_id(0)

    @pl.when(i == 0)
    def _init():
        u_acc[...] = jnp.zeros_like(u_acc)
        kv_acc[...] = jnp.zeros_like(kv_acc)
        z_acc[...] = jnp.zeros_like(z_acc)
        wkT_ref[...] = wqkv_ref[:, D:2 * D].astype(f32).T.astype(bf16)

    @pl.when(i < NS)
    def _phase1():
        x = x_ref[...]
        xT = x.astype(f32).T
        mu = jnp.mean(xT, axis=0, keepdims=True)
        xc = xT - mu
        var = jnp.mean(xc * xc, axis=0, keepdims=True)
        hT = (xc / jnp.sqrt(var + 1e-5)).astype(bf16)
        u_acc[...] += jnp.dot(hT, w1_ref[...], preferred_element_type=f32)
        kT = jnp.dot(wkT_ref[...], xT.astype(bf16), preferred_element_type=f32)
        pkT = _phi(kT)
        zs = pkT[:, 0:128]
        for c in range(1, TS // 128):
            zs = zs + pkT[:, c * 128:(c + 1) * 128]
        z_acc[...] += zs
        pkTb = pkT.astype(bf16)
        v = jnp.dot(x, wqkv_ref[:, 2 * D:3 * D], preferred_element_type=f32).astype(bf16)
        for j in range(NG):
            kv_acc[j] += jnp.dot(pkTb[j * 128:(j + 1) * 128, :], v[:, j * 128:(j + 1) * 128],
                                 preferred_element_type=f32)

    @pl.when(i == NS)
    def _phase2():
        u = u_acc[...] + b1_ref[...].astype(f32)
        gu_ref[...] = jax.nn.gelu(u, approximate=True).astype(bf16)
        r = lax.broadcasted_iota(jnp.int32, (128, 128), 0) // DH
        c = lax.broadcasted_iota(jnp.int32, (128, 128), 1) // DH
        mask = r == c
        zcol = jnp.sum(z_acc[...], axis=1, keepdims=True)
        for j in range(NG):
            kvj = jnp.where(mask, kv_acc[j], 0.0).astype(bf16)
            kvw_ref[j * 128:(j + 1) * 128, :] = jnp.dot(
                kvj, wo_ref[j * 128:(j + 1) * 128, :], preferred_element_type=f32).astype(bf16)
            zmat_ref[j] = jnp.where(mask, zcol[j * 128:(j + 1) * 128, :], 0.0).astype(bf16)

    @pl.when(i >= NS)
    def _phase3():
        x = x_ref[...]
        q = jnp.dot(x, wqkv_ref[:, 0:D], preferred_element_type=f32)
        pq = _phi(q)
        pqb = pq.astype(bf16)
        den = jnp.concatenate(
            [jnp.dot(pqb[:, j * 128:(j + 1) * 128], zmat_ref[j], preferred_element_type=f32)
             for j in range(NG)], axis=1) + 1e-6
        pqn = (pq / den).astype(bf16)
        a = jnp.dot(pqn, kvw_ref[...], preferred_element_type=f32)
        y = jnp.dot(gu_ref[...], w2_ref[...], preferred_element_type=f32)
        y = y + b2_ref[...].astype(f32)
        b = y.T
        g = jax.nn.sigmoid(jnp.sum(x.astype(f32) * gw_ref[...].astype(f32), axis=-1, keepdims=True))
        o_ref[...] = (g * a + (1.0 - g) * b).astype(o_ref.dtype)


@jax.jit
def pallas_gated_mix__linear_attn_block__mixer_token_mlp__prompt_kernel(
        A_x, A_wqkv, A_wo, B_x, B_w1, B_b1, B_w2, B_b2, gate_w):
    x = A_x.reshape(S, D)
    b1 = B_b1.reshape(1, F)
    b2 = B_b2.reshape(1, S)
    gw = gate_w.reshape(1, D)

    def xmap(i):
        return (jnp.where(i < NS, i, i - NS), 0)

    grid_spec = pltpu.PrefetchScalarGridSpec(
        num_scalar_prefetch=0,
        grid=(2 * NS,),
        in_specs=[
            pl.BlockSpec((TS, D), xmap),
            pl.BlockSpec((D, 3 * D), lambda i: (0, 0)),
            pl.BlockSpec((D, D), lambda i: (0, 0)),
            pl.BlockSpec((TS, F), lambda i: (jnp.minimum(i, NS - 1), 0)),
            pl.BlockSpec((1, F), lambda i: (0, 0)),
            pl.BlockSpec((F, TS), lambda i: (0, jnp.maximum(i - NS, 0))),
            pl.BlockSpec((1, TS), lambda i: (0, jnp.maximum(i - NS, 0))),
            pl.BlockSpec((1, D), lambda i: (0, 0)),
        ],
        out_specs=pl.BlockSpec((TS, D), lambda i: (jnp.maximum(i - NS, 0), 0)),
        scratch_shapes=[
            pltpu.VMEM((D, F), jnp.float32),
            pltpu.VMEM((NG, 128, 128), jnp.float32),
            pltpu.VMEM((D, 128), jnp.float32),
            pltpu.VMEM((D, F), jnp.bfloat16),
            pltpu.VMEM((D, D), jnp.bfloat16),
            pltpu.VMEM((NG, 128, 128), jnp.bfloat16),
            pltpu.VMEM((D, D), jnp.bfloat16),
        ],
    )
    out = pl.pallas_call(
        _kernel,
        grid_spec=grid_spec,
        out_shape=jax.ShapeDtypeStruct((S, D), jnp.bfloat16),
        compiler_params=pltpu.CompilerParams(
            dimension_semantics=("arbitrary",),
            vmem_limit_bytes=100 * 1024 * 1024,
        ),
    )(x, A_wqkv, A_wo, B_w1, b1, B_w2, b2, gw)
    return out.reshape(1, S, D)
```

```python
import jax
import jax.numpy as jnp
from jax import lax
import jax.experimental.pallas as pl
import jax.experimental.pallas.tpu as pltpu

S, D, F, DH = 2048, 512, 1792, 16
TS = 256
NS = S // TS
NG = D // 128
FC = 256


def _phi(t):
    return jnp.where(t > 0, t + 1.0, jnp.exp(t)) + 1e-6


def _kernel(x_hbm, wqkv_hbm, wo_hbm, w1_hbm, b1_ref, w2_hbm, b2_ref, gw_ref, o_hbm,
            x_v, wqkv_v, wo_v, w1_buf, w2_buf, o_buf,
            u_acc, kv_acc, z_acc, gu_ref, kvw_ref, zmat_ref, wkT_ref,
            sem_x, sem_w1, sem_w2, sem_o, sem_c):
    f32, bf16 = jnp.float32, jnp.bfloat16

    def x_copy(i, slot):
        return pltpu.make_async_copy(x_hbm.at[pl.ds(i * TS, TS), :], x_v.at[pl.ds(i * TS, TS), :], sem_x.at[slot])

    def w1_copy(i, slot):
        return pltpu.make_async_copy(w1_hbm.at[pl.ds(i * TS, TS), :], w1_buf.at[slot], sem_w1.at[slot])

    def w2_copy(i, slot):
        return pltpu.make_async_copy(w2_hbm.at[:, pl.ds(i * TS, TS)], w2_buf.at[slot], sem_w2.at[slot])

    def o_copy(i, slot):
        return pltpu.make_async_copy(o_buf.at[slot], o_hbm.at[pl.ds(i * TS, TS), :], sem_o.at[slot])

    wqkv_cp = pltpu.make_async_copy(wqkv_hbm, wqkv_v, sem_c.at[0])
    wo_cp = pltpu.make_async_copy(wo_hbm, wo_v, sem_c.at[1])

    x_copy(0, 0).start()
    w1_copy(0, 0).start()
    wqkv_cp.start()
    x_copy(1, 1).start()
    w1_copy(1, 1).start()

    def p1_prep(off):
        x = x_v[pl.ds(off, TS), :]
        xT = x.astype(f32).T
        mu = jnp.mean(xT, axis=0, keepdims=True)
        xc = xT - mu
        var = jnp.mean(xc * xc, axis=0, keepdims=True)
        hT = (xc / jnp.sqrt(var + 1e-5)).astype(bf16)
        return x, xT.astype(bf16), hT

    def p1_attn(x, xTb, first):
        v = jnp.dot(x, wqkv_v[:, 2 * D:3 * D], preferred_element_type=f32).astype(bf16)
        kT = jnp.dot(wkT_ref[...], xTb, preferred_element_type=f32)
        return v, kT

    def p1_kv(v, kT):
        pkT = _phi(kT)
        zs = pkT[:, 0:128]
        for c in range(1, TS // 128):
            zs = zs + pkT[:, c * 128:(c + 1) * 128]
        z_acc[...] += zs
        pkTb = pkT.astype(bf16)
        for j in range(NG):
            kv_acc[j] += jnp.dot(pkTb[j * 128:(j + 1) * 128, :], v[:, j * 128:(j + 1) * 128],
                                 preferred_element_type=f32)

    x_copy(0, 0).wait()
    w1_copy(0, 0).wait()
    x0, xTb0, hT0 = p1_prep(0)
    for c in range(F // FC):
        u_acc[:, c * FC:(c + 1) * FC] = jnp.dot(hT0, w1_buf[0, :, c * FC:(c + 1) * FC],
                                                preferred_element_type=f32)
    kv_acc[...] = jnp.zeros_like(kv_acc)
    z_acc[...] = jnp.zeros_like(z_acc)
    wqkv_cp.wait()
    wo_cp.start()
    wkT_ref[...] = wqkv_v[:, D:2 * D].astype(f32).T.astype(bf16)
    p1_kv(*p1_attn(x0, xTb0, True))

    def phase1(i, carry):
        slot = i % 2
        x_copy(i, slot).wait()
        w1_copy(i, slot).wait()
        x_copy(i + 1, 1 - slot).start()
        w1_copy(i + 1, 1 - slot).start()
        off = pl.multiple_of(i * TS, TS)
        x = x_v[pl.ds(off, TS), :]
        v = jnp.dot(x, wqkv_v[:, 2 * D:3 * D], preferred_element_type=f32).astype(bf16)
        xT = x.astype(f32).T
        kT = jnp.dot(wkT_ref[...], xT.astype(bf16), preferred_element_type=f32)
        mu = jnp.mean(xT, axis=0, keepdims=True)
        xc = xT - mu
        var = jnp.mean(xc * xc, axis=0, keepdims=True)
        hT = (xc / jnp.sqrt(var + 1e-5)).astype(bf16)
        for c in range(F // FC):
            u_acc[:, c * FC:(c + 1) * FC] += jnp.dot(
                hT, w1_buf[slot, :, c * FC:(c + 1) * FC], preferred_element_type=f32)
        p1_kv(v, kT)
        return carry

    lax.fori_loop(1, NS - 1, phase1, 0)

    lslot = (NS - 1) % 2
    x_copy(NS - 1, lslot).wait()
    w1_copy(NS - 1, lslot).wait()
    w2_copy(0, 0).start()
    xl, xTbl, hTl = p1_prep((NS - 1) * TS)
    for c in range(F // FC):
        uc = u_acc[:, c * FC:(c + 1) * FC] + jnp.dot(
            hTl, w1_buf[lslot, :, c * FC:(c + 1) * FC], preferred_element_type=f32)
        uc = uc + b1_ref[c * FC:(c + 1) * FC].astype(f32).reshape(1, FC)
        gu_ref[:, c * FC:(c + 1) * FC] = jax.nn.gelu(uc, approximate=True).astype(bf16)
    p1_kv(*p1_attn(xl, xTbl, False))

    rr = lax.broadcasted_iota(jnp.int32, (128, 128), 0) // DH
    cc = lax.broadcasted_iota(jnp.int32, (128, 128), 1) // DH
    mask = rr == cc
    zcol = jnp.sum(z_acc[...], axis=1, keepdims=True)
    wo_cp.wait()
    for j in range(NG):
        kvj = jnp.where(mask, kv_acc[j], 0.0).astype(bf16)
        kvw_ref[j * 128:(j + 1) * 128, :] = jnp.dot(
            kvj, wo_v[j * 128:(j + 1) * 128, :], preferred_element_type=f32).astype(bf16)
        zmat_ref[j] = jnp.where(mask, zcol[j * 128:(j + 1) * 128, :], 0.0).astype(bf16)

    def phase3(i, carry):
        slot = i % 2
        w2_copy(i, slot).wait()

        @pl.when(i + 1 < NS)
        def _():
            w2_copy(i + 1, 1 - slot).start()

        @pl.when(i >= 2)
        def _():
            o_copy(i - 2, slot).wait()

        off = pl.multiple_of(i * TS, TS)
        x = x_v[pl.ds(off, TS), :]
        q = jnp.dot(x, wqkv_v[:, 0:D], preferred_element_type=f32)
        yA = jnp.dot(gu_ref[...], w2_buf[slot, :, 0:128], preferred_element_type=f32)
        pq = _phi(q)
        pqb = pq.astype(bf16)
        den = jnp.concatenate(
            [jnp.dot(pqb[:, j * 128:(j + 1) * 128], zmat_ref[j], preferred_element_type=f32)
             for j in range(NG)], axis=1) + 1e-6
        yB = jnp.dot(gu_ref[...], w2_buf[slot, :, 128:256], preferred_element_type=f32)
        pqn = (pq / den).astype(bf16)
        a = jnp.dot(pqn, kvw_ref[...], preferred_element_type=f32)
        y = jnp.concatenate([yA, yB], axis=1) + b2_ref[pl.ds(off, TS)].astype(f32).reshape(1, TS)
        b = y.T
        g = jax.nn.sigmoid(jnp.sum(x.astype(f32) * gw_ref[...].astype(f32).reshape(1, D),
                                   axis=-1, keepdims=True))
        o_buf[slot] = (g * a + (1.0 - g) * b).astype(o_buf.dtype)
        o_copy(i, slot).start()
        return carry

    lax.fori_loop(0, NS, phase3, 0)
    o_copy(NS - 2, (NS - 2) % 2).wait()
    o_copy(NS - 1, (NS - 1) % 2).wait()


@jax.jit
def pallas_gated_mix__linear_attn_block__mixer_token_mlp__prompt_kernel(
        A_x, A_wqkv, A_wo, B_x, B_w1, B_b1, B_w2, B_b2, gate_w):
    x = A_x.reshape(S, D)
    any_spec = pl.BlockSpec(memory_space=pl.ANY)
    out = pl.pallas_call(
        _kernel,
        in_specs=[any_spec, any_spec, any_spec, any_spec,
                  pl.BlockSpec((F,), lambda: (0,)),
                  any_spec,
                  pl.BlockSpec((S,), lambda: (0,)),
                  pl.BlockSpec((D,), lambda: (0,))],
        out_specs=any_spec,
        out_shape=jax.ShapeDtypeStruct((S, D), jnp.bfloat16),
        scratch_shapes=[
            pltpu.VMEM((S, D), jnp.bfloat16),
            pltpu.VMEM((D, 3 * D), jnp.bfloat16),
            pltpu.VMEM((D, D), jnp.bfloat16),
            pltpu.VMEM((2, TS, F), jnp.bfloat16),
            pltpu.VMEM((2, F, TS), jnp.bfloat16),
            pltpu.VMEM((2, TS, D), jnp.bfloat16),
            pltpu.VMEM((D, F), jnp.float32),
            pltpu.VMEM((NG, 128, 128), jnp.float32),
            pltpu.VMEM((D, 128), jnp.float32),
            pltpu.VMEM((D, F), jnp.bfloat16),
            pltpu.VMEM((D, D), jnp.bfloat16),
            pltpu.VMEM((NG, 128, 128), jnp.bfloat16),
            pltpu.VMEM((D, D), jnp.bfloat16),
            pltpu.SemaphoreType.DMA((2,)),
            pltpu.SemaphoreType.DMA((2,)),
            pltpu.SemaphoreType.DMA((2,)),
            pltpu.SemaphoreType.DMA((2,)),
            pltpu.SemaphoreType.DMA((2,)),
        ],
        compiler_params=pltpu.CompilerParams(
            vmem_limit_bytes=100 * 1024 * 1024,
        ),
    )(x, A_wqkv, A_wo, B_w1, B_b1, B_w2, B_b2, gate_w)
    return out.reshape(1, S, D)
```
